```python
import os as _os
_os.environ.setdefault("JAX_PLATFORMS", "cpu")
import jax
import jax.numpy as jnp

def _softmax(x, axis=-1):
    return jax.nn.softmax(x, axis=axis)
def _gelu(x):
    return jax.nn.gelu(x, approximate=True)
def _silu(x):
    return jax.nn.silu(x)
def _sigmoid(x):
    return jax.nn.sigmoid(x)
def _layernorm(x, axis=-1, eps=1e-5):
    m = jnp.mean(x, axis=axis, keepdims=True)
    v = jnp.var(x, axis=axis, keepdims=True)
    return (x - m) / jnp.sqrt(v + eps)
def _scatter_add(tgt, idx, src, axis=0):
    return tgt.at[idx].add(src)
def _segment_sum(src, seg, n):
    return jax.ops.segment_sum(src, seg, n)
class _Rng:
    def __init__(self, key):
        self._k = key
    def _next(self):
        self._k, sub = jax.random.split(self._k)
        return sub
    def normal(self, shape):
        return jax.random.normal(self._next(), shape, dtype=jnp.bfloat16)
    def randint(self, lo, hi, shape):
        return jax.random.randint(self._next(), shape, lo, hi, dtype=jnp.int32)
    def uniform(self, shape, lo=0.0, hi=1.0):
        return jax.random.uniform(self._next(), shape, jnp.bfloat16, lo, hi)
    def permutation(self, n):
        return jax.random.permutation(self._next(), n)


kernel_name = 'interleave_layers__sliding_local_dilated__mixer_s_mlp__prompt'

def setup_inputs():
    _rng = _Rng(jax.random.key(int.from_bytes(__import__("os").urandom(4), "little")))
    _w = (lambda a: (lambda t: t.astype(jnp.bfloat16) if jnp.issubdtype(t.dtype, jnp.floating) else t)(jnp.asarray(a)))
    def _A_setup():
        B, S, D = 1, 2048, 448
        return {
            "x": _w((lambda *s: _rng.normal(s) * 0.05)(B, S, D)),
            "wqkv": _w((lambda *s: _rng.normal(s) * 0.05)(D, 3 * D)),
            "wo": _w((lambda *s: _rng.normal(s) * 0.05)(D, D)),
        }
    _A_in = _A_setup()

    def _B_setup():
        B, S, D, F = 1, 2048, 448, 1792
        return {
            "x":  _w((lambda *s: _rng.normal(s) * 0.05)(B, S, D)),
            "w1": _w((lambda *s: _rng.normal(s) * 0.8)(D, D) * (D ** -0.5)),
            "w2": _w((lambda *s: _rng.normal(s) * 0.8)(D, D) * (D ** -0.5)),
            "w3": _w((lambda *s: _rng.normal(s) * 0.8)(D, F) * (D ** -0.5)),
            "w4": _w((lambda *s: _rng.normal(s) * 0.8)(F, D) * (F ** -0.5)),
        }
    _B_in = _B_setup()

    return {
        "A_x": _A_in["x"],
        "A_wqkv": _A_in["wqkv"],
        "A_wo": _A_in["wo"],
        "B_x": _B_in["x"],
        "B_w1": _B_in["w1"],
        "B_w2": _B_in["w2"],
        "B_w3": _B_in["w3"],
        "B_w4": _B_in["w4"],
    }

def reference(A_x, A_wqkv, A_wo, B_x, B_w1, B_w2, B_w3, B_w4):
    def _A_ref(x, wqkv, wo):
        B, S, D = x.shape
        H = 16; Dh = D // H
        W, dil = 8, 2
        qkv = (lambda x, *d: x.transpose(*d))((x @ wqkv).reshape(B, S, 3, H, Dh), 2, 0, 3, 1, 4)
        q, k, v = qkv[0], qkv[1], qkv[2]
        scale = Dh ** -0.5
        pos = jnp.arange(S)
        off = jnp.arange(W) * dil
        idx = pos[:, None] - off[None, :]
        mask = idx >= 0
        idx_c = jnp.where(mask, idx, 0).reshape(-1)
        kg = k[:, :, idx_c, :].reshape(B, H, S, W, Dh)
        vg = v[:, :, idx_c, :].reshape(B, H, S, W, Dh)
        logits = jnp.einsum("bhsd,bhswd->bhsw", q, kg) * scale
        logits = jnp.where(mask[None, None, :, :], logits, -1e9)
        attn = _softmax(logits, axis=-1)
        o = jnp.einsum("bhsw,bhswd->bhsd", attn, vg)
        return (lambda x, *d: x.transpose(*d))(o, 0, 2, 1, 3).reshape(B, S, D) @ wo

    def _B_ref(x, w1, w2, w3, w4):
        B, S, D = x.shape
        h = _gelu(_layernorm(x, axis=-1) @ w1)
        c = D // 4
        g0 = jnp.pad(h[:, :, 0*c:1*c], ((0, 0), (1, 0), (0, 0)))[:, :S, :]
        g1 = jnp.pad(h[:, :, 1*c:2*c], ((0, 0), (0, 1), (0, 0)))[:, 1:, :]
        g2 = jnp.pad(h[:, :, 2*c:3*c], ((0, 0), (2, 0), (0, 0)))[:, :S, :]
        g3 = jnp.pad(h[:, :, 3*c:   ], ((0, 0), (0, 2), (0, 0)))[:, 2:, :]
        hs = jnp.concatenate([g0, g1, g2, g3], axis=-1) @ w2
        x1 = x + hs
        h2 = _gelu(_layernorm(x1, axis=-1) @ w3) @ w4
        return x1 + h2

    x = A_x
    x = x + _A_ref(_layernorm(x, axis=-1), A_wqkv, A_wo)
    x = x + _B_ref(_layernorm(x, axis=-1), B_w1, B_w2, B_w3, B_w4)
    x = x + _A_ref(_layernorm(x, axis=-1), A_wqkv, A_wo)
    x = x + _B_ref(_layernorm(x, axis=-1), B_w1, B_w2, B_w3, B_w4)
    return x
```

```python
import functools
import math

import jax
import jax.numpy as jnp
from jax.experimental import pallas as pl
from jax.experimental.pallas import tpu as pltpu

S, D, F = 2048, 448, 1792
DH, DIL, EPS = 28, 2, 1e-5
T, G = 128, 4
NT, NG = S // T, S // T // G
B, BH = 112, 64
HB, ND, NF = B // 2, D // B, F // BH
F32, BF16, U32 = jnp.float32, jnp.bfloat16, jnp.uint32

_GK, _GC = math.sqrt(2.0 / math.pi), 0.044715
_GA = (_GK * _GC) ** (1.0 / 3.0)

LEVEL = dict(qkv=1, wo=1, w1=1, w2=1, w3=2, w4=1)
BLOCKS = dict(qkv=3 * ND, wo=ND, w1=ND, w2=ND, w3=NF, w4=ND)
STEP = dict(qkv=1, wo=1, w1=1, w2=1, w3=1, w4=1)
CYCLES = dict(qkv=4704, wo=1568, w1=1568, w2=1568, w3=5488, w4=5488)

ORDER = """
qkv0.0 qkv0.1 qkv0.2 qkv0.3a+wo+w1 wo0.0+w2 qkv0.3b+w3 w10.0 wo0.1+w4 w10.1a w20.0 w10.1b
w30.0 w40.0a wo0.2a w40.0b qkv1.0 wo0.2b w10.2a w20.1 w10.2b
w30.1 w40.1a wo0.3a w40.1b qkv1.1 wo0.3b w10.3a w20.2 w10.3b
w30.2 w40.2 qkv1.2 wo1.0 w20.3 w11.0 w30.3 w40.3 qkv1.3 wo1.1 w11.1a w21.0 w11.1b
w31.0 w41.0 wo1.2 w11.2a w21.1 w11.2b w31.1 w41.1 wo1.3 w11.3 w21.2 w21.3
w31.2 w41.2a w31.3 w41.2b w41.3
""".split()
ATT_STEPS = 2 * NT * 8 + 1


def _cat(xs, axis=0):
    return xs[0] if len(xs) == 1 else jnp.concatenate(xs, axis=axis)


def _pack(low, high):
    return pltpu.pack_elementwise([low, high], packed_dtype=BF16)


def _pack_block(x):
    n = x.shape[0] // 2
    return _pack(x[:n], x[n:])


def _unpack_block(words):
    return _cat([pltpu.unpack_elementwise(words, index=i, packed_dtype=BF16, unpacked_dtype=F32)
                 for i in range(2)])


def _blk(i, size=B):
    return slice(i * size, (i + 1) * size)


def _quad(m):
    h = len(m) // 2
    return ([r[:h] for r in m[:h]], [r[h:] for r in m[:h]],
            [r[:h] for r in m[h:]], [r[h:] for r in m[h:]])


def _add(a, b):
    return [[x + y for x, y in zip(r, s)] for r, s in zip(a, b)]


def _sub(a, b):
    return [[x - y for x, y in zip(r, s)] for r, s in zip(a, b)]


def _w_terms(w):
    if len(w) == 1:
        return [w[0][0]]
    w11, w12, w21, w22 = _quad(w)
    return [t for c in (w11, _add(w11, w12), _add(w21, w22), w22, _add(w11, w22),
                        _sub(w21, w11), _sub(w12, w22)) for t in _w_terms(c)]


def _x_terms(x):
    if len(x) == 1:
        return [x[0][0]]
    x11, x12, x21, x22 = _quad(x)
    return [t for c in (_sub(x12, x22), x22, x11, _sub(x21, x11), _add(x11, x22),
                        _add(x11, x12), _add(x21, x22)) for t in _x_terms(c)]


def _products(level, prod, emit, base=0):
    if level == 0:
        emit(0, 0, prod(base))
        yield
        return
    n, h = 7 ** (level - 1), 2 ** (level - 1)
    a, b, c = {}, {}, {}

    def m3(m, t, x): a[m, t] = x
    def m5(m, t, x): b[m, t] = x; emit(m, h + t, a[m, t] + x)
    def m2(m, t, x): c[m, t] = x; a[m, t] = a[m, t] - x
    def m4(m, t, x): b[m, t] = x - b[m, t]; emit(h + m, t, c[m, t] + x)
    def m1(m, t, x): a[m, t] = a[m, t] + x; b[m, t] = b[m, t] + x
    def m6(m, t, x): emit(h + m, h + t, a[m, t] + x)
    def m7(m, t, x): emit(m, t, b[m, t] + x)

    for i, fn in enumerate((m3, m5, m2, m4, m1, m6, m7)):
        yield from _products(level - 1, prod, fn, base + i * n)


def _run(gen):
    for _ in gen:
        pass


def _chain(*gens):
    for gen in gens:
        yield from gen
        yield


def _parse(job):
    part = 0.5 if job[-1] in "ab" else 1
    job = job.rstrip("ab")
    return job[:-3], int(job[-3]), int(job[-1]), part


def _plan(jobs):
    shared, start, end, clock = {}, {}, {}, 0
    for i, job in enumerate(jobs):
        name, _, _, part = _parse(job)
        busy = name in ("w1", "w2", "w3") and i >= jobs.index("w30.0")
        shared[job] = 0 if busy else CYCLES[name] * part
        start[job] = clock
        clock += shared[job]
        end[job] = clock

    def at(table, job, j):
        return table.get(f"{job}.{j // G}{'ab'[j % G // 2]}", table.get(f"{job}.{j // G}"))

    ready, due = [], []
    for layer in range(2):
        for step in range(ATT_STEPS):
            newest = min((min(step // 8, 2 * NT - 1) + 1) // 2 + 1, NT - 1)
            j = min(max((step - 3) // 8 - 1, 0) // 2, NT - 1)
            g = j // G
            ready.append(at(end, f"qkv{layer}", newest) + 300)
            due.append(at(start, f"wo{layer}", j) - 300)
            if layer or g > 1:
                ready[-1] = max(ready[-1], at(end, f"wo{layer}", g * G - 1) if g else at(end, "wo0", NT - 1))
    steps, t = [], 0
    for i in range(len(ready)):
        t = max(t, ready[i])
        rate = min((due[k] - t) / (k - i + 1) for k in range(i, len(ready)))
        rate = max(min(rate, 330), 0)
        lag = -(-(180 if t < start["w30.0"] else 135) * 7 // max(int(rate), 1))
        steps.append((min(t, due[i]), min(max(lag, 4), 14)))
        t += rate
    return shared, steps


def _kernel(x_hbm, w_hbm, o_hbm, xin, xout, raw, ta, tb, td, wts, acts, bufs, isem, wsem, osem):
    lane = jax.lax.broadcasted_iota(jnp.int32, (8, T), 1)
    never = ((lane * (lane + 1)) & 1) == 1

    def after(x, *ys):
        for y in ys:
            x = jnp.where(never, y, x)
        return x

    def hold(ref, value):
        pltpu.store(ref, value, mask=jax.lax.broadcasted_iota(jnp.int32, value.shape, 1) >= 0)

    xs, x2s, x1s, qs, ks, vs, os_, hs, ys = bufs
    pending, latest, trail = [], [], []
    done = set()

    def dot(w, a):
        now = [v for d, v in pending if d <= 0]
        pending[:] = [[d - 1, v] for d, v in pending if d > 0]
        if now:
            head = after(w[:8, :T], *now)
            w = _cat([_cat([head, w[:8, T:]], 1) if w.shape[1] > T else head, w[8:]])
        r = jnp.dot(pltpu.bitcast(w, BF16), pltpu.bitcast(a, BF16), preferred_element_type=F32)
        latest[:] = [r[:8]]
        return r

    def shr(prev, cur, d):
        keep = jnp.broadcast_to(lane[:1] >= T - d, cur.shape)
        return pltpu.roll(cur if prev is None else jnp.where(keep, prev, cur), d, 1)

    def shl(cur, nxt, d):
        keep = jnp.broadcast_to(lane[:1] < d, cur.shape)
        return pltpu.roll(cur if nxt is None else jnp.where(keep, nxt, cur), T - d, 1)

    def x_copy(g):
        return pltpu.make_async_copy(x_hbm.at[:, pl.ds(g * G * T, G * T)], xin.at[g], isem.at[g])

    def w_copy(name):
        return pltpu.make_async_copy(w_hbm[name], raw[name], wsem.at[list(LEVEL).index(name)])

    def qkv_copy(k):
        return pltpu.make_async_copy(
            w_hbm["qkv"].at[_blk(k, D // 2)], raw["qkv"].at[_blk(k, D // 2)], wsem.at[len(LEVEL) + k])

    def o_copy(p, b):
        return pltpu.make_async_copy(
            xout.at[p, _blk(b)], o_hbm.at[_blk(b), pl.ds(p * 2 * T, 2 * T)], osem.at[p * ND + b])

    def store_terms(name, nm, nk, get, spread=0):
        n = 2 ** LEVEL[name]
        pm, pk = nm // n, nk // n
        for c in range(pm):
            w = [[[get(m * pm + c, k * pk + i) for i in range(pk)] for k in range(n)] for m in range(n)]
            if isinstance(w[0][0][0], tuple):
                even, odd = (_w_terms([[_cat([p[e] for p in x], 1) for x in row] for row in w])
                             for e in range(2))
                words = [_pack(*x) for x in zip(even, odd)]
            else:
                words = [pltpu.bitcast(x.astype(BF16), U32)
                         for x in _w_terms([[_cat(x, 1) for x in row] for row in w])]
            rows = words[0].shape[0]
            for i, x in enumerate(words):
                hold(wts[name].at[i, _blk(c, rows)], x)
            if spread:
                for r in range(c * rows, (c + 1) * rows, 8):
                    stored = [wts[name][i, r:r + 8, :T] for i in range(len(words))]
                    pending.append([spread * (r + 8) // (pm * rows), after(*stored)])
            yield

    def transpose_in(rows_of, m):
        for k in range(ND):
            rows = rows_of(k)
            ta[k, :m] = _cat([rows, jnp.zeros((T - B, rows.shape[1]), F32)]).T[:m]
            yield

    def even_odd(m, k):
        return _cat([ta[k, pl.ds(m * B + i, HB, stride=2), :] for i in range(2)])

    def prep_plain(name):
        yield from transpose_in(lambda k: raw[name][_blk(k), :].astype(F32), D)
        yield from store_terms(name, ND, ND, even_odd)

    def prep_qkv():
        yield from transpose_in(lambda k: raw["qkv"][_blk(k), :].astype(F32), 3 * D)
        yield from store_terms("qkv", 3 * ND, ND, lambda m, k: tuple(
            _cat([ta[k, pl.ds(m // ND * D + e * (D // 2) + m % ND * 7 + d, 8, stride=DH), :]
                  for d in range(7)]) for e in range(2)))

    def prep_wo():
        w = _cat([raw["wo"][...].astype(F32), jnp.zeros((D, 4 * T - D), F32)], 1)
        for c in range(4):
            tb[0, c, :D] = w[:, c * T:(c + 1) * T]
            for row in range(0, D, 8):
                for e in range(2):
                    src = (8 * e + row % 16 // 2) * DH + row // 16
                    dst = row // B * B + 2 * ((row % B + e) % HB) + row % B // HB
                    tb[1, c, pl.ds(dst, 4, stride=4), :] = tb[0, c, pl.ds(src, 4, stride=DH), :]
        yield
        yield from transpose_in(lambda k: _cat([tb[1, c, _blk(k)] for c in range(4)], 1), D)
        yield from store_terms("wo", ND, ND, even_odd)

    def prep_w3():
        for k in range(ND):
            rows = _cat([raw["w3"][_blk(k), :], jnp.zeros((T - B, F), BF16)])
            td[k, :F // 2] = pltpu.bitcast(rows.T, U32)
            yield
        yield from store_terms("w3", NF, ND, lambda m, k: tuple(
            _unpack_block(td[k, pl.ds(m * BH // 2 + e, BH // 4, stride=2), :]) for e in range(2)), 60)

    def prep_w4():
        yield from store_terms("w4", ND, 2, lambda m, k: _unpack_block(
            pltpu.bitcast(raw["w4"][_blk(m), _blk(k, F // 2)], U32)))

    def slot(name, g):
        return acts[name][g % len(acts[name])]

    def put_terms(name, g, sub, c, x):
        for i, term in enumerate(_x_terms(x)):
            words = _pack_block(term)
            at = (i, _blk(c, words.shape[0]))
            if name == "w4":
                hold(slot(name, g)[sub].at[at], words)
            else:
                slot(name, g)[sub][at] = words
            first = words if i == 0 else first
        return first[-8:]

    def operands(name, g, get):
        n = 2 ** LEVEL[name]
        for sub in range(G // n):
            for c in range(ND // n):
                yield put_terms(name, g, sub, c, [[get(sub * n + t, k * (ND // n) + c)
                                                   for t in range(n)] for k in range(n)])

    def matmul(name, g, emit, chunk_done=lambda sub, c: None):
        n, step, size = 2 ** LEVEL[name], STEP[name], BH if name == "w3" else B
        pm = BLOCKS[name] // n

        def stationary(sub, i):
            a = slot(name, g)[sub][i]
            if name == "w4":
                return a
            pad = jnp.zeros(((T - B) // 2, T), U32)
            return _cat([x for k in range(a.shape[0] // HB) for x in (a[_blk(k, HB)], pad)])

        for sub in range(G // n):
            for c in range(0, pm, step):
                def out(m, t, x):
                    for i in range(step):
                        emit(sub * n + t, m * pm + c + i, x[_blk(i, size)])

                products = _products(LEVEL[name], lambda i: dot(
                    wts[name][i, c * size // 2:(c + step) * size // 2], stationary(sub, i)), out)
                for _ in range(7 ** LEVEL[name] - 1):
                    next(products)
                    yield
                _run(products)
                for i in range(step):
                    chunk_done(sub, c + i)
                yield

    def fold(x):
        parts = [x[8 * i:8 * i + 8] for i in range(x.shape[0] // 8)]
        return functools.reduce(jnp.add, parts[0::2]) + functools.reduce(jnp.add, parts[1::2])

    def accumulate(sums, t, x):
        new = (fold(x), fold(x * x))
        sums[t] = tuple(map(jnp.add, sums[t], new)) if t in sums else new

    def mean_var(sums, t):
        mean, square = (jnp.broadcast_to(jnp.sum(x, axis=0, keepdims=True) * (1.0 / D), (8, T))
                        for x in sums.pop(t))
        return mean, jnp.maximum(square - mean * mean, 0.0)

    def scaled(x, mean, scale):
        return x * _cat([scale] * (B // 8)) - _cat([mean * scale] * (B // 8))

    def normed_operands(name, g, sums, src, gain=1.0):
        mv = [mean_var(sums, t) for t in range(G)]
        rs = [jax.lax.rsqrt(var + EPS) for _, var in mv]
        rs = rs if gain == 1.0 else [r * gain for r in rs]
        return list(operands(name, g, lambda t, b: scaled(src[g * G + t][_blk(b)], mv[t][0], rs[t])))

    def load_x(g):
        sums = {}
        for t in range(G):
            for b in range(ND):
                x = _unpack_block(pltpu.bitcast(xin[g, _blk(b), _blk(t, T)], U32))
                hold(xs[g * G + t].at[_blk(b)], x)
                accumulate(sums, t, x)
        return normed_operands("qkv", g, sums, xs)

    pace = [0]

    def attention(layer):
        lg1, lgs, p0, p1, p1s = ({} for _ in range(5))
        todo = []

        def rows(hh, d):
            return slice(16 * d + 8 * hh, 16 * d + 8 * hh + 8)

        def paced(x):
            return after(x, *trail[-pace[0]]) if len(trail) >= pace[0] else x

        def tick(d):
            if d < DH - 1 and todo:
                todo.pop(0)()

        def qk(j, hh):
            assert ("qkv", layer, min(j + 1, NT - 1), 3 * ND - 1) in done
            a0, a1 = [None] * 4, [None] * 4
            for d in range(DH):
                r = rows(hh, d)
                q0, k0 = qs[j][r], ks[j][r]
                kp = ks[j - 1][r] if j > 0 else None
                q1 = shl(q0, qs[j + 1][r] if j + 1 < NT else None, 4 * DIL)
                kg = paced(k0)
                for b in range(4):
                    kb = k0 if b == 0 else shr(kp, kg, b * DIL)
                    t0, t1 = q0 * kb, q1 * kb
                    a0[b] = t0 if d == 0 else a0[b] + t0
                    a1[b] = t1 if d == 0 else a1[b] + t1
                trail.append([a0[d % 4], a1[d % 4]])
                if d % 7 == 6:
                    tick(d)
                    yield
            lg1[j, hh] = a1

            def shift_logits():
                lgs[j, hh] = [shr(lg1[j - 1, hh][b] if j > 0 else None, a1[b], 4 * DIL) for b in range(4)]

            def softmax():
                lg = [x * (DH ** -0.5) for x in a0 + lgs.pop((j, hh))]
                if j == 0:
                    lg = [x if w == 0 else jnp.where(lane >= w * DIL, x, -1e9) for w, x in enumerate(lg)]
                top = functools.reduce(jnp.maximum, lg)
                e = [jnp.exp(x - top) for x in lg]
                inv = 1.0 / functools.reduce(jnp.add, e)
                p = [x * inv for x in e]
                p0[j, hh], p1[j, hh] = p[:4], p[4:]

            def shift_weights():
                if j > 0:
                    p1s[j - 1, hh] = [shl(p1[j - 1, hh][b], p1[j, hh][b], 4 * DIL) for b in range(4)]
                else:
                    p1s[-1, hh] = shl(functools.reduce(jnp.add, p1[0, hh]), None, 4 * DIL)
                if j == NT - 1:
                    p1s[j, hh] = [shl(p1[j, hh][b], None, 4 * DIL) for b in range(4)]

            todo.extend([shift_logits, softmax, shift_weights])

        def pv(j, hh):
            pa, pb = p0.pop((j, hh)), p1s.pop((j, hh))
            lag = pace[0]
            y0, y1 = {}, {}
            if j == 0:
                first = [jnp.broadcast_to(vs[0][rows(hh, d)][:, :1], (8, T)) for d in range(DH)]

            def finish(ds):
                for d in ds:
                    prev = ys[(j - 1) % 2][rows(hh, d)] if j > 0 else p1s[-1, hh] * first[d]
                    hold(os_[j].at[rows(hh, d)], y0[d] + shr(prev, y1[d], 4 * DIL))
                    done.add(("o", layer, j, hh, d))

            for d in range(DH):
                v0 = vs[j][rows(hh, d)]
                vp = vs[j - 1][rows(hh, d)] if j > 0 else first[d]
                vg = paced(v0)
                vb = [v0] + [shr(vp, vg, b * DIL) for b in range(1, 4)]
                y0[d] = (pa[0] * vb[0] + pa[1] * vb[1]) + (pa[2] * vb[2] + pa[3] * vb[3])
                y1[d] = (pb[0] * vb[0] + pb[1] * vb[1]) + (pb[2] * vb[2] + pb[3] * vb[3])
                trail.append([y0[d]])
                if j + 1 < NT:
                    hold(ys[j % 2].at[rows(hh, d)], y1[d])
                if d >= lag:
                    finish([d - lag])
                if d % 7 == 6:
                    tick(d)
                    yield
            todo.extend(functools.partial(finish, range(DH - lag + i * lag // 3, DH - lag + (i + 1) * lag // 3))
                        for i in range(3))

        for j in range(NT + 1):
            for unit, i in ((qk, j), (pv, j - 1)):
                if 0 <= i < NT:
                    yield from unit(i, 0)
                    yield from unit(i, 1)
        while todo:
            todo.pop(0)()

    norm2 = {}

    def job_qkv(layer, g):
        def emit(t, b, x):
            hold((qs, ks, vs)[b // ND][g * G + t].at[_blk(b % ND)], x)
            done.add(("qkv", layer, g * G + t, b))
        yield from matmul("qkv", g, emit)

    def pre_wo(layer, g):
        def get(t, b):
            assert ("o", layer, g * G + t, 1, DH - 1) in done
            return os_[g * G + t][_blk(b)]
        yield from operands("wo", g, get)

    def job_wo(layer, g):
        j0, sums, scales = g * G, {}, []

        def emit(t, b, r):
            x2 = xs[j0 + t][_blk(b)] + r
            hold(x2s[j0 + t].at[_blk(b)], x2)
            accumulate(sums, t, x2)

        def norm(pair, c):
            if c == ND // 2 - 1:
                for t in (2 * pair, 2 * pair + 1):
                    mean, var = mean_var(sums, t)
                    r = jax.lax.rsqrt(var + EPS)
                    norm2[j0 + t] = (mean, r)
                    scales.append(r * jax.lax.rsqrt(var * r * r + EPS) * _GA)
                next(normed), next(normed)

        normed = operands("w1", g, lambda t, b: scaled(x2s[j0 + t][_blk(b)], norm2[j0 + t][0], scales[t]))
        yield from matmul("wo", g, emit, norm)

    def gelu(y):
        return y + y * jnp.tanh(y * (y * y + _GK / _GA))

    def job_w1(layer, g):
        def emit(t, b, r):
            hold(hs[g * G + t].at[_blk(b)], gelu(r))
            done.add(("h", layer, g * G + t, b))
        yield from matmul("w1", g, emit)

    def pre_w2(layer, g):
        def shifted(t, b):
            def part(j):
                assert not 0 <= j < NT or ("h", layer, j, b) in done
                return hs[j][_blk(b)] if 0 <= j < NT else jnp.zeros((B, T), F32)
            j = g * G + t
            if b % 2 == 0:
                return shr(part(j - 1), part(j), 1 + b // 2)
            return shl(part(j), part(j + 1), 1 + b // 2)
        yield from operands("w2", g, shifted)

    def job_w2(layer, g):
        j0, sums = g * G, {}

        def emit(t, b, r):
            x1 = scaled(x2s[j0 + t][_blk(b)], *norm2[j0 + t]) + r * (0.5 / _GA)
            hold(x1s[j0 + t].at[_blk(b)], x1)
            accumulate(sums, t, x1)

        yield from matmul("w2", g, emit)
        normed_operands("w3", g, sums, x1s, _GA)

    def job_w3(layer, g):
        hidden = {}

        def emit(t, b, r):
            hidden[t, b] = gelu(r)

        def chunk_done(sub, c):
            for pair in range(2):
                for b in (c, NF // 4 + c):
                    put_terms("w4", g, pair, b, [[hidden.pop((2 * pair + t, k * (NF // 2) + b))
                                                  for t in range(2)] for k in range(2)])

        yield from matmul("w3", g, emit, chunk_done)

    def job_w4(layer, g):
        j0, sums = g * G, {}

        def emit(t, b, r):
            x = (x2s[j0 + t][_blk(b)] + x1s[j0 + t][_blk(b)]) + r * (0.5 / _GA)
            if layer == 0:
                hold(xs[j0 + t].at[_blk(b)], x)
                accumulate(sums, t, x)
            else:
                xout[(j0 + t) // 2, _blk(b), _blk(t % 2, T)] = pltpu.bitcast(_pack_block(x), BF16)

        def chunk_done(pair, c):
            if layer == 1:
                o_copy(j0 // 2 + pair, c).start()
                o_copy(j0 // 2 + pair, ND // 2 + c).start()

        yield from matmul("w4", g, emit, chunk_done)
        if layer == 0:
            normed_operands("qkv", g, sums, xs)

    jobs = dict(qkv=job_qkv, wo=job_wo, w1=job_w1, w2=job_w2, w3=job_w3, w4=job_w4)
    preps = dict(wo=prep_wo, w1=lambda: prep_plain("w1"), w2=lambda: prep_plain("w2"),
                 w3=prep_w3, w4=prep_w4)
    names = [item.split("+")[0] for item in ORDER]
    shared, plan = _plan(names)
    att = _chain(attention(0), attention(1))

    first = [qkv_copy(k) for k in range(2)] + [x_copy(0)]
    for copy in first:
        copy.start()
    for copy in first:
        copy.wait()
    for g in range(1, NG):
        x_copy(g).start()
    load_x(0)
    _run(prep_qkv())

    clock, paused, running = 0, False, {}
    for pos, item in enumerate(ORDER):
        job, *extra = item.split("+")
        name, layer, g, part = _parse(job)
        if "wo" in extra:
            for n in preps:
                w_copy(n).wait()
        streams = [(_chain(*(preps[n]() for n in extra)), 5 * len(extra))] if extra else []
        if job[-1] != "b":
            running[name] = jobs[name](layer, g)
            if name == "wo":
                running["o"] = pre_wo(layer, g)
        if name == "wo":
            for _ in range(int(4 * part)):
                next(running["o"])
        if pos + 1 < len(names) and names[pos + 1][:-3] == "w2":
            streams.append((pre_w2(*_parse(names[pos + 1])[1:3]), 4))
        n = 2 ** LEVEL[name]
        total = int(7 ** LEVEL[name] * (G // n) * (BLOCKS[name] // n // STEP[name]) * part)
        cut = total - 2 if pos + 1 < len(ORDER) and "+wo" in ORDER[pos + 1] else total
        taken = [0] * len(streams)
        for i in range(total):
            next(running[name])
            if pos == 0 and i + 1 == total // 2:
                for k in range(1, NG):
                    x_copy(k).wait()
                for w in preps:
                    w_copy(w).start()
                early = load_x(1) + load_x(2)
                pending.extend([(k + 1) * (total // 2 - 2) // len(early), v] for k, v in enumerate(early))
                load_x(3)
            if paused and i == 0:
                trail.extend([latest[:]] * 16)
            if i < cut:
                while plan and plan[0][0] <= clock + shared[job] * (i + 1) / total:
                    pace[0] = plan.pop(0)[1]
                    next(att)
            elif i == cut:
                pending.extend([0, pltpu.bitcast(v, U32)] for row in trail[-4:] for v in row)
            for k, (gen, steps) in enumerate(streams):
                while taken[k] < steps * (i + 1) // total:
                    taken[k] += 1
                    next(gen, None)
        for gen, _ in streams:
            _run(gen)
        if job[-1] != "a":
            _run(running.pop(name))
        clock += shared[job]
        paused = shared[job] == 0
    for p in range(NT // 2):
        for b in range(ND):
            o_copy(p, b).wait()


@jax.jit
def pallas_interleave_layers__sliding_local_dilated__mixer_s_mlp__prompt_kernel(
        A_x, A_wqkv, A_wo, B_x, B_w1, B_w2, B_w3, B_w4):
    del B_x
    weights = dict(qkv=A_wqkv, wo=A_wo, w1=B_w1, w2=B_w2, w3=B_w3, w4=B_w4.T)
    depth = {n: F if n == "w4" else D for n in LEVEL}
    side = {n: 2 ** level for n, level in LEVEL.items()}
    tile = pltpu.VMEM((D, T), F32)
    hbm = pl.BlockSpec(memory_space=pl.ANY)
    out = pl.pallas_call(
        _kernel,
        out_shape=jax.ShapeDtypeStruct((D, S), BF16),
        in_specs=[hbm, {n: hbm for n in weights}],
        out_specs=hbm,
        scratch_shapes=[
            pltpu.VMEM((NG, D, G * T), BF16),
            pltpu.VMEM((NT // 2, D, 2 * T), BF16),
            {n: pltpu.VMEM(w.shape, BF16) for n, w in weights.items()},
            pltpu.VMEM((ND, 3 * D + 32, T), F32),
            pltpu.VMEM((2, 4, D + 32, T), F32),
            pltpu.VMEM((ND, F // 2 + 8, T), U32),
            {n: pltpu.VMEM((7 ** LEVEL[n], dict(qkv=3 * D, w3=F).get(n, D) // side[n] // 2,
                            (F if n == "w4" else ND * T) // side[n]), U32) for n in LEVEL},
            {n: [[pltpu.VMEM((7 ** LEVEL[n], depth[n] // side[n] // 2, T), U32)] * (G // side[n])]
             * (NG if n == "qkv" else 2) for n in LEVEL},
            [[tile] * NT] * 8 + [[tile] * 2],
            pltpu.SemaphoreType.DMA((NG,)),
            pltpu.SemaphoreType.DMA((len(LEVEL) + 2,)),
            pltpu.SemaphoreType.DMA((NT // 2 * ND,)),
        ],
        compiler_params=pltpu.CompilerParams(vmem_limit_bytes=120 * 2 ** 20),
        name="fused_block",
    )(A_x.reshape(S, D).T, weights)
    return out.T.reshape(1, S, D)
```
